```python
import os as _os
_os.environ.setdefault("JAX_PLATFORMS", "cpu")
import jax
import jax.numpy as jnp

def _softmax(x, axis=-1):
    return jax.nn.softmax(x, axis=axis)
def _gelu(x):
    return jax.nn.gelu(x, approximate=True)
def _silu(x):
    return jax.nn.silu(x)
def _sigmoid(x):
    return jax.nn.sigmoid(x)
def _layernorm(x, axis=-1, eps=1e-5):
    m = jnp.mean(x, axis=axis, keepdims=True)
    v = jnp.var(x, axis=axis, keepdims=True)
    return (x - m) / jnp.sqrt(v + eps)
def _scatter_add(tgt, idx, src, axis=0):
    return tgt.at[idx].add(src)
def _segment_sum(src, seg, n):
    return jax.ops.segment_sum(src, seg, n)
class _Rng:
    def __init__(self, key):
        self._k = key
    def _next(self):
        self._k, sub = jax.random.split(self._k)
        return sub
    def normal(self, shape):
        return jax.random.normal(self._next(), shape, dtype=jnp.bfloat16)
    def randint(self, lo, hi, shape):
        return jax.random.randint(self._next(), shape, lo, hi, dtype=jnp.int32)
    def uniform(self, shape, lo=0.0, hi=1.0):
        return jax.random.uniform(self._next(), shape, jnp.bfloat16, lo, hi)
    def permutation(self, n):
        return jax.random.permutation(self._next(), n)


kernel_name = 'interleave_layers__linear_kernel_hedgehog__dense_activation_silu__prompt'

def setup_inputs():
    _rng = _Rng(jax.random.key(int.from_bytes(__import__("os").urandom(4), "little")))
    _w = (lambda a: (lambda t: t.astype(jnp.bfloat16) if jnp.issubdtype(t.dtype, jnp.floating) else t)(jnp.asarray(a)))
    def _A_setup():
        B, S, D, H = 1, 2048, 640, 32
        Dh = D // H
        return {
            "x": _w((lambda *s: _rng.normal(s) * 0.05)(B, S, D)),
            "wqkv": _w((lambda *s: _rng.normal(s) * 0.4)(D, 3 * D)),
            "w_phi": _w((lambda *s: _rng.normal(s) * 0.4)(H, Dh, Dh) * (Dh ** -0.5)),
            "wo": _w((lambda *s: _rng.normal(s) * 0.05)(D, D)),
        }
    _A_in = _A_setup()

    def _B_setup():
        B, S, D, F = 1, 2048, 640, 1728
        return {
            "x": _w((lambda *s: _rng.normal(s) * 0.05)(B, S, D)),
            "w1": _w((lambda *s: _rng.normal(s) * 1.6)(D, F) * (D ** -0.5)),
            "w2": _w((lambda *s: _rng.normal(s) * 1.6)(F, D) * (F ** -0.5)),
        }
    _B_in = _B_setup()

    return {
        "A_x": _A_in["x"],
        "A_wqkv": _A_in["wqkv"],
        "A_w_phi": _A_in["w_phi"],
        "A_wo": _A_in["wo"],
        "B_x": _B_in["x"],
        "B_w1": _B_in["w1"],
        "B_w2": _B_in["w2"],
    }

def reference(A_x, A_wqkv, A_w_phi, A_wo, B_x, B_w1, B_w2):
    def _A_ref(x, wqkv, w_phi, wo):
        B, S, D = x.shape
        H = 32; Dh = D // H
        qkv = (lambda x, *d: x.transpose(*d))((x @ wqkv).reshape(B, S, 3, H, Dh), 2, 0, 3, 1, 4)
        q, k, v = qkv[0], qkv[1], qkv[2]
        pq = jnp.einsum("bhsd,hdf->bhsf", q, w_phi)
        pk = jnp.einsum("bhsd,hdf->bhsf", k, w_phi)
        phi_q = jnp.concatenate([_softmax(pq, axis=-1), _softmax(-pq, axis=-1)], axis=-1)
        phi_k = jnp.concatenate([_softmax(pk, axis=-1), _softmax(-pk, axis=-1)], axis=-1)
        kv = jnp.einsum("bhsf,bhsd->bhfd", phi_k, v)
        z  = jnp.einsum("bhsf->bhf", phi_k)
        num = jnp.einsum("bhqf,bhfd->bhqd", phi_q, kv)
        den = jnp.einsum("bhqf,bhf->bhq", phi_q, z)[..., None] + 1e-6
        o = num / den
        return (lambda x, *d: x.transpose(*d))(o, 0, 2, 1, 3).reshape(B, S, D) @ wo

    def _B_ref(x, w1, w2):
        h = jnp.einsum("bsd,df->bsf", x, w1)
        h = _silu(h)
        out = jnp.einsum("bsf,fd->bsd", h, w2)
        return out

    x = A_x
    x = x + _A_ref(_layernorm(x, axis=-1), A_wqkv, A_w_phi, A_wo)
    x = x + _B_ref(_layernorm(x, axis=-1), B_w1, B_w2)
    x = x + _A_ref(_layernorm(x, axis=-1), A_wqkv, A_w_phi, A_wo)
    x = x + _B_ref(_layernorm(x, axis=-1), B_w1, B_w2)
    return x
```

```python
import functools
import jax
import jax.numpy as jnp
from jax import lax
import jax.experimental.pallas as pl
import jax.experimental.pallas.tpu as pltpu

f32, bf16 = jnp.float32, jnp.bfloat16
NT = (((1,), (1,)), ((), ()))
TN = (((0,), (0,)), ((), ()))

D = 640
H = 32
DH = 20
NG = 16
GR = 40
NP = 5
KVR = 48


def _layernorm(x):
    m = jnp.mean(x, axis=-1, keepdims=True)
    xc = x - m
    v = jnp.mean(xc * xc, axis=-1, keepdims=True)
    return xc * lax.rsqrt(v + 1e-5)


def _tile_allreduce(m, op):
    m = op(m, pltpu.roll(m, 2, 1))
    return op(m, pltpu.roll(m, 4, 1))


def _dual_softmax(a, R):
    a4 = a.reshape(NG, NP, 8, R)
    mx = _tile_allreduce(jnp.max(a4, axis=1), jnp.maximum)[:, None]
    mn = _tile_allreduce(jnp.min(a4, axis=1), jnp.minimum)[:, None]
    eP = jnp.exp(a4 - mx)
    eN = jnp.exp(mn - a4)
    sP = _tile_allreduce(jnp.sum(eP, axis=1), jnp.add)
    sN = _tile_allreduce(jnp.sum(eN, axis=1), jnp.add)
    return eP * (1.0 / sP)[:, None], eN * (1.0 / sN)[:, None]


def _group_phi(phiP, phiN, g, R):
    return jnp.concatenate([phiP[g].reshape(GR, R), phiN[g].reshape(GR, R)], axis=0).astype(bf16)


def _kernel(x_hbm, wqkv_hbm, g_hbm, wo_hbm, w1_hbm, w2_hbm, out_ref,
            g_v, wqkv_v, wo_v, w1_v, w2_v, xin_v,
            p_scr, pv_scr, wt_scr, wop_scr, xs_scr, phiq_scr, kvacc_scr, kvl_scr, ot_scr, sems,
            *, R, T):
    p = pl.program_id(0)
    t = pl.program_id(1)

    def cp(src, dst, i):
        return pltpu.make_async_copy(src, dst, sems.at[i])

    def cp_x(tt):
        return cp(x_hbm.at[pl.ds(tt * R, R), :], xin_v.at[tt], 5 + tt)

    @pl.when((p == 0) & (t == 0))
    def _prep():
        cp(g_hbm, g_v, 0).start()
        cp(wqkv_hbm, wqkv_v, 1).start()
        cp(wo_hbm, wo_v, 2).start()
        cp(g_hbm, g_v, 0).wait()
        srow = lax.broadcasted_iota(jnp.int32, (8, D), 0)
        dcol = lax.broadcasted_iota(jnp.int32, (8, D), 1)
        hh = srow & 1
        fsub = srow >> 1
        g = g_v[...].astype(f32)
        gtiles = []
        for pp in range(NP):
            rows = [jnp.broadcast_to(g[4 * pp + i: 4 * pp + i + 1, :], (8, D)) for i in range(4)]
            gt = jnp.where(fsub == 0, rows[0], jnp.where(fsub == 1, rows[1], jnp.where(fsub == 2, rows[2], rows[3])))
            gtiles.append(gt)
        for grp in range(NG):
            lo = (2 * grp + hh) * DH
            colmask = (dcol >= lo) & (dcol < lo + DH)
            for pp in range(NP):
                r0 = GR * grp + 8 * pp
                p_scr[r0: r0 + 8, :] = jnp.where(colmask, gtiles[pp], 0.0)
                pv_scr[r0: r0 + 8, :] = jnp.where(dcol == lo + 4 * pp + fsub, 1.0, 0.0).astype(f32)
        cp(wqkv_hbm, wqkv_v, 1).wait()
        cp(wo_hbm, wo_v, 2).wait()
        for tt in range(T):
            cp_x(tt).start()
        cp(w1_hbm, w1_v, 3).start()
        cp(w2_hbm, w2_v, 4).start()
        for j in range(4):
            k0 = (160 * j // 128) * 128
            a_p = p_scr[160 * j: 160 * (j + 1), k0: k0 + 256].astype(bf16)
            a_v = pv_scr[160 * j: 160 * (j + 1), k0: k0 + 256].astype(bf16)
            for part in range(2):
                w = wqkv_v[:, part * D + k0: part * D + k0 + 256]
                wt_scr[part * D + 160 * j: part * D + 160 * (j + 1), :] = lax.dot_general(
                    a_p, w, NT, preferred_element_type=f32).astype(bf16)
            w = wqkv_v[:, 2 * D + k0: 2 * D + k0 + 256]
            wt_scr[2 * D + 160 * j: 2 * D + 160 * (j + 1), :] = lax.dot_general(
                a_v, w, NT, preferred_element_type=f32).astype(bf16)
            wop_scr[160 * j: 160 * (j + 1), :] = jnp.dot(
                a_v, wo_v[k0: k0 + 256, :], preferred_element_type=f32).astype(bf16)
        kvacc_scr[...] = jnp.zeros(kvacc_scr.shape, f32)

    @pl.when((p >= 1) & (t == 0))
    def _finalize():
        @pl.when(p == 1)
        def _():
            cp(w1_hbm, w1_v, 3).wait()
            cp(w2_hbm, w2_v, 4).wait()
        rr = lax.broadcasted_iota(jnp.int32, (KVR, 2 * GR), 0)
        cc = lax.broadcasted_iota(jnp.int32, (KVR, 2 * GR), 1)
        mask = (rr & 1) == (cc & 1)
        for g in range(NG):
            kvl_scr[g] = jnp.where(mask, kvacc_scr[g], 0.0).astype(bf16)
        kvacc_scr[...] = jnp.zeros(kvacc_scr.shape, f32)

    @pl.when(p >= 1)
    def _a2b():
        x = xs_scr[t]
        for gg in range(NG // 2):
            os = []
            for g in (2 * gg, 2 * gg + 1):
                nd = jnp.dot(kvl_scr[g], phiq_scr[t, g], preferred_element_type=f32)
                num = nd[0:GR].reshape(NP, 8, R)
                den = nd[GR:KVR] + 1e-6
                os.append((num * (1.0 / den)[None]).reshape(GR, R))
            ot_scr[2 * GR * gg: 2 * GR * (gg + 1), :] = jnp.concatenate(os, axis=0).astype(bf16)
        attn = lax.dot_general(ot_scr[...], wop_scr[...], TN, preferred_element_type=f32)
        x = x + attn
        xn = _layernorm(x).astype(bf16)
        h = jnp.dot(xn, w1_v[...], preferred_element_type=f32)
        h = h * (1.0 / (1.0 + jnp.exp(-h)))
        y = jnp.dot(h.astype(bf16), w2_v[...], preferred_element_type=f32)
        xs_scr[t] = x + y

    @pl.when(p == 0)
    def _load():
        cp_x(t).wait()
        xs_scr[t] = xin_v[t].astype(f32)

    @pl.when(p <= 1)
    def _a1():
        xn = _layernorm(xs_scr[t]).astype(bf16)
        qkvT = lax.dot_general(wt_scr[...], xn, NT, preferred_element_type=f32)
        qP, qN = _dual_softmax(qkvT[0:D], R)
        for g in range(NG):
            phiq_scr[t, g] = _group_phi(qP, qN, g, R)
        kP, kN = _dual_softmax(qkvT[D:2 * D], R)
        ones = jnp.ones((KVR - GR, R), f32)
        for g in range(NG):
            phik = _group_phi(kP, kN, g, R)
            va = jnp.concatenate([qkvT[2 * D + GR * g: 2 * D + GR * (g + 1)], ones], axis=0).astype(bf16)
            kvacc_scr[g] += lax.dot_general(va, phik, NT, preferred_element_type=f32)

    @pl.when(p == 2)
    def _store():
        out_ref[...] = xs_scr[t].astype(out_ref.dtype)


@jax.jit
def pallas_interleave_layers__linear_kernel_hedgehog__dense_activation_silu__prompt_kernel(A_x, A_wqkv, A_w_phi, A_wo, B_x, B_w1, B_w2):
    R = 512
    B, S, _ = A_x.shape
    F = B_w1.shape[1]
    T = S // R
    x2 = A_x.reshape(S, D)
    g = jnp.transpose(A_w_phi, (2, 0, 1)).reshape(DH, D)
    kern = functools.partial(_kernel, R=R, T=T)
    hbm = pl.BlockSpec(memory_space=pltpu.HBM)
    out = pl.pallas_call(
        kern,
        grid=(3, T),
        in_specs=[hbm] * 6,
        out_specs=pl.BlockSpec((R, D), lambda p, t: (jnp.where(p == 2, t, 0), 0)),
        out_shape=jax.ShapeDtypeStruct((S, D), A_x.dtype),
        scratch_shapes=[
            pltpu.VMEM((DH, D), bf16),
            pltpu.VMEM((D, 3 * D), bf16),
            pltpu.VMEM((D, D), bf16),
            pltpu.VMEM((D, F), bf16),
            pltpu.VMEM((F, D), bf16),
            pltpu.VMEM((T, R, D), bf16),
            pltpu.VMEM((D, D), f32),
            pltpu.VMEM((D, D), f32),
            pltpu.VMEM((3 * D, D), bf16),
            pltpu.VMEM((D, D), bf16),
            pltpu.VMEM((T, R, D), f32),
            pltpu.VMEM((T, NG, 2 * GR, R), bf16),
            pltpu.VMEM((NG, KVR, 2 * GR), f32),
            pltpu.VMEM((NG, KVR, 2 * GR), bf16),
            pltpu.VMEM((D, R), bf16),
            pltpu.SemaphoreType.DMA((5 + T,)),
        ],
        compiler_params=pltpu.CompilerParams(
            dimension_semantics=("arbitrary", "arbitrary"),
            vmem_limit_bytes=100 * 1024 * 1024),
    )(x2, A_wqkv, g, A_wo, B_w1, B_w2)
    return out.reshape(B, S, D)
```

```python
import functools
import jax
import jax.numpy as jnp
from jax import lax
import jax.experimental.pallas as pl
import jax.experimental.pallas.tpu as pltpu

f32, bf16 = jnp.float32, jnp.bfloat16
NT = (((1,), (1,)), ((), ()))
TN = (((0,), (0,)), ((), ()))

D = 640
H = 32
DH = 20
NG = 16
GR = 40
NP = 5
KVR = 48


def _layernorm(x):
    m = jnp.mean(x, axis=-1, keepdims=True)
    xc = x - m
    v = jnp.mean(xc * xc, axis=-1, keepdims=True)
    return xc * lax.rsqrt(v + 1e-5)


def _tile_allreduce(m, op):
    m = op(m, pltpu.roll(m, 2, 1))
    return op(m, pltpu.roll(m, 4, 1))


def _dual_softmax(a, R):
    a4 = a.reshape(NG, NP, 8, R)
    mx = _tile_allreduce(jnp.max(a4, axis=1), jnp.maximum)[:, None]
    mn = _tile_allreduce(jnp.min(a4, axis=1), jnp.minimum)[:, None]
    eP = jnp.exp(a4 - mx)
    eN = jnp.exp(mn - a4)
    sP = _tile_allreduce(jnp.sum(eP, axis=1), jnp.add)
    sN = _tile_allreduce(jnp.sum(eN, axis=1), jnp.add)
    return eP * (1.0 / sP)[:, None], eN * (1.0 / sN)[:, None]


def _group_phi(phiP, phiN, g, R):
    return jnp.concatenate([phiP[g].reshape(GR, R), phiN[g].reshape(GR, R)], axis=0).astype(bf16)


def _kernel(x_hbm, wqkv_hbm, g_hbm, wo_hbm, w1_hbm, w2_hbm, out_ref,
            g_v, wqkv_v, wo_v, w1_v, w2_v, xin_v,
            p_scr, pv_scr, wt_scr, wop_scr, xs_scr, phiq_scr, kvacc_scr, kvl_scr, ot_scr, sems,
            *, R, T):
    p = pl.program_id(0)
    t = pl.program_id(1)

    def cp(src, dst, i):
        return pltpu.make_async_copy(src, dst, sems.at[i])

    def cp_x(tt):
        return cp(x_hbm.at[pl.ds(tt * R, R), :], xin_v.at[tt], 7 + tt)

    def cp_w(part):
        return cp(wqkv_hbm.at[:, pl.ds(part * D, D)], wqkv_v.at[:, pl.ds(part * D, D)], 1 + part)

    @pl.when((p == 0) & (t == 0))
    def _prep():
        cp(g_hbm, g_v, 0).start()
        for part in range(3):
            cp_w(part).start()
        cp(wo_hbm, wo_v, 4).start()
        cp(g_hbm, g_v, 0).wait()
        srow = lax.broadcasted_iota(jnp.int32, (8, D), 0)
        dcol = lax.broadcasted_iota(jnp.int32, (8, D), 1)
        hh = srow & 1
        fsub = srow >> 1
        g = g_v[...].astype(f32)
        gtiles = []
        for pp in range(NP):
            rows = [jnp.broadcast_to(g[4 * pp + i: 4 * pp + i + 1, :], (8, D)) for i in range(4)]
            gt = jnp.where(fsub == 0, rows[0], jnp.where(fsub == 1, rows[1], jnp.where(fsub == 2, rows[2], rows[3])))
            gtiles.append(gt)
        for grp in range(NG):
            lo = (2 * grp + hh) * DH
            colmask = (dcol >= lo) & (dcol < lo + DH)
            for pp in range(NP):
                r0 = GR * grp + 8 * pp
                p_scr[r0: r0 + 8, :] = jnp.where(colmask, gtiles[pp], 0.0)
                pv_scr[r0: r0 + 8, :] = jnp.where(dcol == lo + 4 * pp + fsub, 1.0, 0.0).astype(f32)
        def krange(c):
            k0 = (2 * GR * c // 128) * 128
            kw = ((2 * GR * c + 2 * GR - 1) // 128) * 128 - k0 + 128
            return k0, kw
        for part in range(3):
            cp_w(part).wait()
            P = p_scr if part < 2 else pv_scr
            for c in range(NG // 2):
                k0, kw = krange(c)
                a = P[2 * GR * c: 2 * GR * (c + 1), k0: k0 + kw].astype(bf16)
                w = wqkv_v[:, part * D + k0: part * D + k0 + kw]
                wt_scr[part * D + 2 * GR * c: part * D + 2 * GR * (c + 1), :] = lax.dot_general(
                    a, w, NT, preferred_element_type=f32).astype(bf16)
        cp(wo_hbm, wo_v, 4).wait()
        for tt in range(T):
            cp_x(tt).start()
        cp(w1_hbm, w1_v, 5).start()
        cp(w2_hbm, w2_v, 6).start()
        for c in range(NG // 2):
            k0, kw = krange(c)
            a_v = pv_scr[2 * GR * c: 2 * GR * (c + 1), k0: k0 + kw].astype(bf16)
            wop_scr[2 * GR * c: 2 * GR * (c + 1), :] = jnp.dot(
                a_v, wo_v[k0: k0 + kw, :], preferred_element_type=f32).astype(bf16)
        kvacc_scr[...] = jnp.zeros(kvacc_scr.shape, f32)

    @pl.when((p >= 1) & (t == 0))
    def _finalize():
        @pl.when(p == 1)
        def _():
            cp(w1_hbm, w1_v, 5).wait()
            cp(w2_hbm, w2_v, 6).wait()
        rr = lax.broadcasted_iota(jnp.int32, (KVR, 2 * GR), 0)
        cc = lax.broadcasted_iota(jnp.int32, (KVR, 2 * GR), 1)
        mask = (rr & 1) == (cc & 1)
        for g in range(NG):
            kvl_scr[g] = jnp.where(mask, kvacc_scr[g], 0.0).astype(bf16)
        kvacc_scr[...] = jnp.zeros(kvacc_scr.shape, f32)

    @pl.when(p >= 1)
    def _a2b():
        x = xs_scr[t]
        for gg in range(NG // 2):
            os = []
            for g in (2 * gg, 2 * gg + 1):
                nd = jnp.dot(kvl_scr[g], phiq_scr[t, g], preferred_element_type=f32)
                num = nd[0:GR].reshape(NP, 8, R)
                den = nd[GR:KVR] + 1e-6
                os.append((num * (1.0 / den)[None]).reshape(GR, R))
            ot_scr[2 * GR * gg: 2 * GR * (gg + 1), :] = jnp.concatenate(os, axis=0).astype(bf16)
        attn = lax.dot_general(ot_scr[...], wop_scr[...], TN, preferred_element_type=f32)
        x = x + attn
        xn = _layernorm(x).astype(bf16)
        h = jnp.dot(xn, w1_v[...], preferred_element_type=f32)
        h = h * (1.0 / (1.0 + jnp.exp(-h)))
        y = jnp.dot(h.astype(bf16), w2_v[...], preferred_element_type=f32)
        xs_scr[t] = x + y

    @pl.when(p == 0)
    def _load():
        cp_x(t).wait()
        xs_scr[t] = xin_v[t].astype(f32)

    @pl.when(p <= 1)
    def _a1():
        xn = _layernorm(xs_scr[t]).astype(bf16)
        qkvT = lax.dot_general(wt_scr[...], xn, NT, preferred_element_type=f32)
        qP, qN = _dual_softmax(qkvT[0:D], R)
        for g in range(NG):
            phiq_scr[t, g] = _group_phi(qP, qN, g, R)
        kP, kN = _dual_softmax(qkvT[D:2 * D], R)
        ones = jnp.ones((KVR - GR, R), f32)
        for g in range(NG):
            phik = _group_phi(kP, kN, g, R)
            va = jnp.concatenate([qkvT[2 * D + GR * g: 2 * D + GR * (g + 1)], ones], axis=0).astype(bf16)
            kvacc_scr[g] += lax.dot_general(va, phik, NT, preferred_element_type=f32)

    @pl.when(p == 2)
    def _store():
        out_ref[...] = xs_scr[t].astype(out_ref.dtype)


@jax.jit
def pallas_interleave_layers__linear_kernel_hedgehog__dense_activation_silu__prompt_kernel(A_x, A_wqkv, A_w_phi, A_wo, B_x, B_w1, B_w2):
    R = 512
    B, S, _ = A_x.shape
    F = B_w1.shape[1]
    T = S // R
    x2 = A_x.reshape(S, D)
    g = jnp.transpose(A_w_phi, (2, 0, 1)).reshape(DH, D)
    kern = functools.partial(_kernel, R=R, T=T)
    hbm = pl.BlockSpec(memory_space=pltpu.HBM)
    out = pl.pallas_call(
        kern,
        grid=(3, T),
        in_specs=[hbm] * 6,
        out_specs=pl.BlockSpec((R, D), lambda p, t: (jnp.where(p == 2, t, 0), 0)),
        out_shape=jax.ShapeDtypeStruct((S, D), A_x.dtype),
        scratch_shapes=[
            pltpu.VMEM((DH, D), bf16),
            pltpu.VMEM((D, 3 * D), bf16),
            pltpu.VMEM((D, D), bf16),
            pltpu.VMEM((D, F), bf16),
            pltpu.VMEM((F, D), bf16),
            pltpu.VMEM((T, R, D), bf16),
            pltpu.VMEM((D, D), f32),
            pltpu.VMEM((D, D), f32),
            pltpu.VMEM((3 * D, D), bf16),
            pltpu.VMEM((D, D), bf16),
            pltpu.VMEM((T, R, D), f32),
            pltpu.VMEM((T, NG, 2 * GR, R), bf16),
            pltpu.VMEM((NG, KVR, 2 * GR), f32),
            pltpu.VMEM((NG, KVR, 2 * GR), bf16),
            pltpu.VMEM((D, R), bf16),
            pltpu.SemaphoreType.DMA((7 + T,)),
        ],
        compiler_params=pltpu.CompilerParams(
            dimension_semantics=("arbitrary", "arbitrary"),
            vmem_limit_bytes=64 * 1024 * 1024),
    )(x2, A_wqkv, g, A_wo, B_w1, B_w2)
    return out.reshape(B, S, D)
```
